```python
import os as _os
_os.environ.setdefault("JAX_PLATFORMS", "cpu")
import jax
import jax.numpy as jnp

def _softmax(x, axis=-1):
    return jax.nn.softmax(x, axis=axis)
def _gelu(x):
    return jax.nn.gelu(x, approximate=True)
def _silu(x):
    return jax.nn.silu(x)
def _sigmoid(x):
    return jax.nn.sigmoid(x)
def _layernorm(x, axis=-1, eps=1e-5):
    m = jnp.mean(x, axis=axis, keepdims=True)
    v = jnp.var(x, axis=axis, keepdims=True)
    return (x - m) / jnp.sqrt(v + eps)
def _scatter_add(tgt, idx, src, axis=0):
    return tgt.at[idx].add(src)
def _segment_sum(src, seg, n):
    return jax.ops.segment_sum(src, seg, n)
class _Rng:
    def __init__(self, key):
        self._k = key
    def _next(self):
        self._k, sub = jax.random.split(self._k)
        return sub
    def normal(self, shape):
        return jax.random.normal(self._next(), shape, dtype=jnp.bfloat16)
    def randint(self, lo, hi, shape):
        return jax.random.randint(self._next(), shape, lo, hi, dtype=jnp.int32)
    def uniform(self, shape, lo=0.0, hi=1.0):
        return jax.random.uniform(self._next(), shape, jnp.bfloat16, lo, hi)
    def permutation(self, n):
        return jax.random.permutation(self._next(), n)


kernel_name = 'concat_heads__gqa_block_cached__gqa_block_cached__near_ridge'

def setup_inputs():
    _rng = _Rng(jax.random.key(int.from_bytes(__import__("os").urandom(4), "little")))
    _w = (lambda a: (lambda t: t.astype(jnp.bfloat16) if jnp.issubdtype(t.dtype, jnp.floating) else t)(jnp.asarray(a)))
    def _A_setup():
        B, Sq, D = 8, 128, 576
        Hq, Hkv, Sk, Dh = 32, 16, 512, 128
        assert Hq % Hkv == 0, (Hq, Hkv)
        return {
            "x": _w((lambda *s: _rng.normal(s) * 0.8)(B, Sq, D)),
            "k_cache": _w((lambda *s: _rng.normal(s) * 0.8)(B, Hkv, Sk, Dh)),
            "v_cache": _w((lambda *s: _rng.normal(s) * 0.05)(B, Hkv, Sk, Dh)),
            "wq": _w((lambda *s: _rng.normal(s) * 0.8)(D, Hq * Dh) * (D ** -0.5)),
            "wo": _w((lambda *s: _rng.normal(s) * 0.05)(Hq * Dh, D) * ((Hq * Dh) ** -0.5)),
        }
    _A_in = _A_setup()

    def _B_setup():
        B, Sq, D = 8, 128, 576
        Hq, Hkv, Sk, Dh = 32, 16, 512, 128
        assert Hq % Hkv == 0, (Hq, Hkv)
        return {
            "x": _w((lambda *s: _rng.normal(s) * 0.8)(B, Sq, D)),
            "k_cache": _w((lambda *s: _rng.normal(s) * 0.8)(B, Hkv, Sk, Dh)),
            "v_cache": _w((lambda *s: _rng.normal(s) * 0.05)(B, Hkv, Sk, Dh)),
            "wq": _w((lambda *s: _rng.normal(s) * 0.8)(D, Hq * Dh) * (D ** -0.5)),
            "wo": _w((lambda *s: _rng.normal(s) * 0.05)(Hq * Dh, D) * ((Hq * Dh) ** -0.5)),
        }
    _B_in = _B_setup()

    return {
        "A_x": _A_in["x"],
        "A_k_cache": _A_in["k_cache"],
        "A_v_cache": _A_in["v_cache"],
        "A_wq": _A_in["wq"],
        "A_wo": _A_in["wo"],
        "B_x": _B_in["x"],
        "B_k_cache": _B_in["k_cache"],
        "B_v_cache": _B_in["v_cache"],
        "B_wq": _B_in["wq"],
        "B_wo": _B_in["wo"],
    }

def reference(A_x, A_k_cache, A_v_cache, A_wq, A_wo, B_x, B_k_cache, B_v_cache, B_wq, B_wo):
    def _A_ref(x, k_cache, v_cache, wq, wo):
        B, Sq, D = x.shape
        Hq, Dh = 32, 128
        Hkv = k_cache.shape[1]
        rep = Hq // Hkv
        q = (lambda x, *d: x.transpose(*d))((x @ wq).reshape(B, Sq, Hq, Dh), 0, 2, 1, 3)
        k = jnp.repeat(k_cache, rep, axis=1)
        v = jnp.repeat(v_cache, rep, axis=1)
        scores = jnp.einsum("bhqd,bhkd->bhqk", q, k) * (Dh ** -0.5)
        p = _softmax(scores, axis=-1)
        o = jnp.einsum("bhqk,bhkd->bhqd", p, v)
        return (lambda x, *d: x.transpose(*d))(o, 0, 2, 1, 3).reshape(B, Sq, Hq * Dh) @ wo

    def _B_ref(x, k_cache, v_cache, wq, wo):
        B, Sq, D = x.shape
        Hq, Dh = 32, 128
        Hkv = k_cache.shape[1]
        rep = Hq // Hkv
        q = (lambda x, *d: x.transpose(*d))((x @ wq).reshape(B, Sq, Hq, Dh), 0, 2, 1, 3)
        k = jnp.repeat(k_cache, rep, axis=1)
        v = jnp.repeat(v_cache, rep, axis=1)
        scores = jnp.einsum("bhqd,bhkd->bhqk", q, k) * (Dh ** -0.5)
        p = _softmax(scores, axis=-1)
        o = jnp.einsum("bhqk,bhkd->bhqd", p, v)
        return (lambda x, *d: x.transpose(*d))(o, 0, 2, 1, 3).reshape(B, Sq, Hq * Dh) @ wo

    a = _A_ref(A_x, A_k_cache, A_v_cache, A_wq, A_wo)
    b = _B_ref(B_x, B_k_cache, B_v_cache, B_wq, B_wo)
    return jnp.concatenate([a, b], axis=-1)
```

```python
import functools
import math

import jax
import jax.numpy as jnp
from jax import lax
import jax.experimental.pallas as pl
import jax.experimental.pallas.tpu as pltpu

_NT = (((1,), (1,)), ((), ()))


def _make_kernel(nb, Sq, Dh, rep, n_h):
    c = (Dh ** -0.5) * math.log2(math.e)

    def kernel(xa_ref, ka_ref, va_ref, wqa_ref, woa_ref,
               xb_ref, kb_ref, vb_ref, wqb_ref, wob_ref,
               out_ref, acca_ref, accb_ref):
        h = pl.program_id(0)
        bb = pl.program_id(1)
        rows = pl.ds(pl.multiple_of(bb * (nb * Sq), nb * Sq), nb * Sq)

        @pl.when(h == 0)
        def _():
            acca_ref[rows, :] = jnp.zeros((nb * Sq, acca_ref.shape[1]), jnp.float32)
            accb_ref[rows, :] = jnp.zeros((nb * Sq, accb_ref.shape[1]), jnp.float32)

        def one(x_ref, k_ref, v_ref, wq_ref, wo_ref, acc_ref):
            q = jnp.dot(x_ref[...], wq_ref[...], preferred_element_type=jnp.float32)
            q = (q * c).astype(jnp.bfloat16)
            os = []
            for j in range(nb):
                qj = q[j * Sq:(j + 1) * Sq]
                qs = jnp.concatenate(
                    [qj[:, r * Dh:(r + 1) * Dh] for r in range(rep)], axis=0)
                s = lax.dot_general(qs, k_ref[j, 0], _NT,
                                    preferred_element_type=jnp.float32)
                m = jnp.max(s, axis=-1, keepdims=True)
                p = jnp.exp2(s - m)
                l = jnp.sum(p, axis=-1, keepdims=True)
                o = jnp.dot(p.astype(jnp.bfloat16), v_ref[j, 0],
                            preferred_element_type=jnp.float32)
                o = (o / l).astype(jnp.bfloat16)
                os.append(jnp.concatenate(
                    [o[r * Sq:(r + 1) * Sq] for r in range(rep)], axis=1))
            o_all = jnp.concatenate(os, axis=0)
            acc_ref[rows, :] += jnp.dot(o_all, wo_ref[...],
                                        preferred_element_type=jnp.float32)

        one(xa_ref, ka_ref, va_ref, wqa_ref, woa_ref, acca_ref)
        one(xb_ref, kb_ref, vb_ref, wqb_ref, wob_ref, accb_ref)

        @pl.when(h == n_h - 1)
        def _():
            out_ref[...] = jnp.concatenate(
                [acca_ref[rows, :], accb_ref[rows, :]], axis=1).astype(out_ref.dtype)

    return kernel


@functools.partial(jax.jit, static_argnames=("nb",))
def _impl(A_x, A_k_cache, A_v_cache, A_wq, A_wo,
          B_x, B_k_cache, B_v_cache, B_wq, B_wo, nb=4):
    B, Sq, D = A_x.shape
    _, Hkv, Sk, Dh = A_k_cache.shape
    Hq = A_wq.shape[1] // Dh
    rep = Hq // Hkv
    n_bb = B // nb

    xa = A_x.reshape(B * Sq, D)
    xb = B_x.reshape(B * Sq, D)

    x_spec = pl.BlockSpec((nb * Sq, D), lambda h, bb: (bb, 0))
    kv_spec = pl.BlockSpec((nb, 1, Sk, Dh), lambda h, bb: (bb, h, 0, 0))
    wq_spec = pl.BlockSpec((D, rep * Dh), lambda h, bb: (0, h))
    wo_spec = pl.BlockSpec((rep * Dh, D), lambda h, bb: (h, 0))
    out_spec = pl.BlockSpec(
        (nb * Sq, 2 * D), lambda h, bb: (jnp.where(h == Hkv - 1, bb, 0), 0))

    out = pl.pallas_call(
        _make_kernel(nb, Sq, Dh, rep, Hkv),
        grid=(Hkv, n_bb),
        in_specs=[x_spec, kv_spec, kv_spec, wq_spec, wo_spec] * 2,
        out_specs=out_spec,
        out_shape=jax.ShapeDtypeStruct((B * Sq, 2 * D), A_x.dtype),
        scratch_shapes=[pltpu.VMEM((B * Sq, D), jnp.float32),
                        pltpu.VMEM((B * Sq, D), jnp.float32)],
        compiler_params=pltpu.CompilerParams(
            dimension_semantics=("arbitrary", "arbitrary"),
            vmem_limit_bytes=100 * 1024 * 1024),
    )(xa, A_k_cache, A_v_cache, A_wq, A_wo,
      xb, B_k_cache, B_v_cache, B_wq, B_wo)
    return out.reshape(B, Sq, 2 * D)


@jax.jit
def pallas_concat_heads__gqa_block_cached__gqa_block_cached__near_ridge_kernel(
    A_x: jax.Array,
    A_k_cache: jax.Array,
    A_v_cache: jax.Array,
    A_wq: jax.Array,
    A_wo: jax.Array,
    B_x: jax.Array,
    B_k_cache: jax.Array,
    B_v_cache: jax.Array,
    B_wq: jax.Array,
    B_wo: jax.Array,
):
    return _impl(A_x, A_k_cache, A_v_cache, A_wq, A_wo,
                 B_x, B_k_cache, B_v_cache, B_wq, B_wo)
```

```python
import functools
import math

import jax
import jax.numpy as jnp
from jax import lax
import jax.experimental.pallas as pl
import jax.experimental.pallas.tpu as pltpu

_NT = (((1,), (1,)), ((), ()))


def _make_kernel(B, Sq, D, Sk, Dh, rep, n_h, qplan, nq, dma_pos, chunks, stage):
    c = (Dh ** -0.5) * math.log2(math.e)
    M = B * Sq
    W = rep * Dh
    MC = M // nq
    n_ch = len(chunks) - 1

    def kernel(xta_hbm, ka_hbm, va_hbm, wqa_hbm, wota_hbm,
               xtb_hbm, kb_hbm, vb_hbm, wqb_hbm, wotb_hbm,
               out_hbm,
               xt_buf, x_buf, k_buf, v_buf, wq_buf, wo_buf, q_buf, acc_ref, out_buf,
               x_sem, kv_sem, kv0_sem, wq_sem, wo_sem, out_sem):
        xt_hbm = (xta_hbm, xtb_hbm)
        k_hbm = (ka_hbm, kb_hbm)
        v_hbm = (va_hbm, vb_hbm)
        wq_hbm = (wqa_hbm, wqb_hbm)
        wot_hbm = (wota_hbm, wotb_hbm)

        def x_copy(blk):
            return pltpu.make_async_copy(xt_hbm[blk], xt_buf.at[blk], x_sem.at[blk])

        def k_copy(h, slot, blk):
            return pltpu.make_async_copy(k_hbm[blk].at[:, h], k_buf.at[slot, blk],
                                         kv_sem.at[slot, blk, 0])

        def v_copy(h, slot, blk):
            return pltpu.make_async_copy(v_hbm[blk].at[:, h], v_buf.at[slot, blk],
                                         kv_sem.at[slot, blk, 1])

        def kv0_copies(ci):
            b0, b1 = chunks[ci], chunks[ci + 1]
            out = []
            for blk in (0, 1):
                out.append(pltpu.make_async_copy(
                    k_hbm[blk].at[pl.ds(b0, b1 - b0), 0],
                    k_buf.at[0, blk, pl.ds(b0, b1 - b0)], kv0_sem.at[ci, blk, 0]))
                out.append(pltpu.make_async_copy(
                    v_hbm[blk].at[pl.ds(b0, b1 - b0), 0],
                    v_buf.at[0, blk, pl.ds(b0, b1 - b0)], kv0_sem.at[ci, blk, 1]))
            return out

        def wq_copy(h, slot, blk):
            return pltpu.make_async_copy(
                wq_hbm[blk].at[:, pl.ds(pl.multiple_of(h * W, W), W)],
                wq_buf.at[slot, blk], wq_sem.at[slot, blk])

        def wo_copy(h, slot, blk):
            return pltpu.make_async_copy(
                wot_hbm[blk].at[:, pl.ds(pl.multiple_of(h * W, W), W)],
                wo_buf.at[slot, blk], wo_sem.at[slot, blk])

        def out_copy(j):
            return pltpu.make_async_copy(out_buf.at[pl.ds(j * Sq, Sq)],
                                         out_hbm.at[pl.ds(j * Sq, Sq)], out_sem.at[j])

        def qproj(slot, blk, ci):
            q = jnp.dot(x_buf[blk, ci * MC:(ci + 1) * MC, :], wq_buf[slot, blk],
                        preferred_element_type=jnp.float32)
            q_buf[slot, blk, ci * MC:(ci + 1) * MC, :] = (q * c).astype(jnp.bfloat16)

        def qk(slot, blk, j):
            qs = jnp.concatenate(
                [q_buf[slot, blk, j * Sq:(j + 1) * Sq, r * Dh:(r + 1) * Dh]
                 for r in range(rep)], axis=0)
            return lax.dot_general(qs, k_buf[slot, blk, j], _NT,
                                   preferred_element_type=jnp.float32)

        def softmax(s):
            m = jnp.max(s, axis=-1, keepdims=True)
            p = jnp.exp2(s - m)
            l = jnp.sum(p, axis=-1, keepdims=True)
            return p.astype(jnp.bfloat16), l

        def pv(p, l, slot, blk, j):
            o = jnp.dot(p, v_buf[slot, blk, j], preferred_element_type=jnp.float32)
            o = (o / l).astype(jnp.bfloat16)
            return jnp.concatenate(
                [o[r * Sq:(r + 1) * Sq] for r in range(rep)], axis=1)

        def oproj(o, slot, blk, j):
            acc_ref[blk * D:(blk + 1) * D, j * Sq:(j + 1) * Sq] += lax.dot_general(
                wo_buf[slot, blk], o, _NT, preferred_element_type=jnp.float32)

        def emit_out(j):
            out_buf[j * Sq:(j + 1) * Sq, :] = (
                acc_ref[:, j * Sq:(j + 1) * Sq].T.astype(out_buf.dtype))
            out_copy(j).start()

        units = [(blk, j) for j in range(B) for blk in (0, 1)]
        n = len(units)

        def start_next(h, slot):
            for blk in (0, 1):
                k_copy(h + 1, 1 - slot, blk).start()
                v_copy(h + 1, 1 - slot, blk).start()
                wo_copy(h + 1, 1 - slot, blk).start()

            @pl.when(h + 2 < n_h)
            def _():
                for blk in (0, 1):
                    wq_copy(h + 2, slot, blk).start()

        def head(h, slot, first, last):
            if first:
                for cp in kv0_copies(0):
                    cp.wait()
            else:
                for blk in (0, 1):
                    k_copy(h, slot, blk).wait()
                    v_copy(h, slot, blk).wait()
            for blk in (0, 1):
                wo_copy(h, slot, blk).wait()
            if not last:
                for blk in (0, 1):
                    wq_copy(h + 1, 1 - slot, blk).wait()
            s = {0: qk(slot, *units[0])}
            o_prev = None
            for u in range(n):
                if u + 1 < n:
                    if first and units[u + 1][0] == 0 and units[u + 1][1] in chunks[1:-1]:
                        ci = chunks.index(units[u + 1][1])
                        for cp in kv0_copies(ci):
                            cp.wait()
                    s[u + 1] = qk(slot, *units[u + 1])
                p, l = softmax(s.pop(u))
                if o_prev is not None:
                    oproj(o_prev, slot, *units[u - 1])
                    if last and units[u - 1][0] == 1:
                        emit_out(units[u - 1][1])
                if not last:
                    for (pos, blk, ci) in qplan:
                        if pos == 2 * u:
                            qproj(1 - slot, blk, ci)
                    if u == (dma_pos if not first else 2 * chunks[-2]):
                        start_next(h, slot)
                o_prev = pv(p, l, slot, *units[u])
                if not last:
                    for (pos, blk, ci) in qplan:
                        if pos == 2 * u + 1:
                            qproj(1 - slot, blk, ci)
            oproj(o_prev, slot, *units[n - 1])
            if last:
                emit_out(units[n - 1][1])
            else:
                for (pos, blk, ci) in qplan:
                    if pos == 2 * n:
                        qproj(1 - slot, blk, ci)

        x_copy(0).start()
        wq_copy(0, 0, 0).start()
        if stage == 0:
            x_copy(1).start()
            wq_copy(0, 0, 1).start()
        acc_ref[...] = jnp.zeros(acc_ref.shape, jnp.float32)
        if stage == 1:
            x_copy(1).start()
            wq_copy(0, 0, 1).start()
        x_copy(0).wait()
        if stage == 2:
            x_copy(1).start()
            wq_copy(0, 0, 1).start()
        for cp in kv0_copies(0):
            cp.start()
        for blk in (0, 1):
            wo_copy(0, 0, blk).start()
        for blk in (0, 1):
            wq_copy(1, 1, blk).start()
        for blk in (0, 1):
            if blk == 1:
                x_copy(blk).wait()
                for ci in range(1, n_ch):
                    for cp in kv0_copies(ci):
                        cp.start()
            for j in range(B):
                x_buf[blk, j * Sq:(j + 1) * Sq, :] = xt_buf[blk, j].T
            wq_copy(0, 0, blk).wait()
            for ci in range(nq):
                qproj(0, blk, ci)

        head(0, 0, True, False)

        def body(h, carry):
            slot = lax.rem(h, 2)
            head(h, slot, False, False)
            return carry

        lax.fori_loop(1, n_h - 1, body, 0)
        head(n_h - 1, (n_h - 1) % 2, False, True)
        for j in range(B):
            out_copy(j).wait()

    return kernel


@functools.partial(jax.jit, static_argnames=("qplan", "nq", "dma_pos", "nobc", "chunks", "stage"))
def _impl(A_x, A_k_cache, A_v_cache, A_wq, A_wo,
          B_x, B_k_cache, B_v_cache, B_wq, B_wo,
          qplan=((26,0,0),(27,0,1),(28,0,2),(29,0,3),(30,1,0),(31,1,1),(32,1,2),(32,1,3)), nq=4, dma_pos=4, nobc=True,
          chunks=(0, 2, 5, 8), stage=0):
    B, Sq, D = A_x.shape
    _, Hkv, Sk, Dh = A_k_cache.shape
    Hq = A_wq.shape[1] // Dh
    rep = Hq // Hkv
    W = rep * Dh
    dt = A_x.dtype

    xta = jnp.transpose(A_x, (0, 2, 1))
    xtb = jnp.transpose(B_x, (0, 2, 1))
    wota = A_wo.T
    wotb = B_wo.T

    any_spec = pl.BlockSpec(memory_space=pl.ANY)
    out = pl.pallas_call(
        _make_kernel(B, Sq, D, Sk, Dh, rep, Hkv, qplan, nq, dma_pos, chunks, stage),
        in_specs=[any_spec] * 10,
        out_specs=any_spec,
        out_shape=jax.ShapeDtypeStruct((B * Sq, 2 * D), dt),
        scratch_shapes=[
            pltpu.VMEM((2, B, D, Sq), dt),
            pltpu.VMEM((2, B * Sq, D), dt),
            pltpu.VMEM((2, 2, B, Sk, Dh), dt),
            pltpu.VMEM((2, 2, B, Sk, Dh), dt),
            pltpu.VMEM((2, 2, D, W), dt),
            pltpu.VMEM((2, 2, D, W), dt),
            pltpu.VMEM((2, 2, B * Sq, W), dt),
            pltpu.VMEM((2 * D, B * Sq), jnp.float32),
            pltpu.VMEM((B * Sq, 2 * D), dt),
            pltpu.SemaphoreType.DMA((2,)),
            pltpu.SemaphoreType.DMA((2, 2, 2)),
            pltpu.SemaphoreType.DMA((len(chunks) - 1, 2, 2)),
            pltpu.SemaphoreType.DMA((2, 2)),
            pltpu.SemaphoreType.DMA((2, 2)),
            pltpu.SemaphoreType.DMA((B,)),
        ],
        compiler_params=pltpu.CompilerParams(
            vmem_limit_bytes=100 * 1024 * 1024,
            disable_bounds_checks=nobc),
    )(xta, A_k_cache, A_v_cache, A_wq, wota,
      xtb, B_k_cache, B_v_cache, B_wq, wotb)
    return out.reshape(B, Sq, 2 * D)


@jax.jit
def pallas_concat_heads__gqa_block_cached__gqa_block_cached__near_ridge_kernel(
    A_x: jax.Array,
    A_k_cache: jax.Array,
    A_v_cache: jax.Array,
    A_wq: jax.Array,
    A_wo: jax.Array,
    B_x: jax.Array,
    B_k_cache: jax.Array,
    B_v_cache: jax.Array,
    B_wq: jax.Array,
    B_wo: jax.Array,
):
    return _impl(A_x, A_k_cache, A_v_cache, A_wq, A_wo,
                 B_x, B_k_cache, B_v_cache, B_wq, B_wo)
```

```python
import functools
import math

import jax
import jax.numpy as jnp
from jax import lax
import jax.experimental.pallas as pl
import jax.experimental.pallas.tpu as pltpu

_NT = (((1,), (1,)), ((), ()))

_NQ = 4
_QPLAN = ((26, 0, 0), (27, 0, 1), (28, 0, 2), (29, 0, 3),
          (30, 1, 0), (31, 1, 1), (32, 1, 2), (32, 1, 3))
_DMA_POS = 4
_CHUNKS = (0, 2, 5, 8)
_OD = 2
_OSL = 2


def _make_kernel(B, Sq, D, Sk, Dh, rep, n_h):
    c = (Dh ** -0.5) * math.log2(math.e)
    M = B * Sq
    W = rep * Dh
    MC = M // _NQ
    chunks = _CHUNKS
    n_ch = len(chunks) - 1

    def kernel(xta_hbm, ka_hbm, va_hbm, wqa_hbm, wota_hbm,
               xtb_hbm, kb_hbm, vb_hbm, wqb_hbm, wotb_hbm,
               out_hbm,
               xt_buf, x_buf, k_buf, v_buf, wq_buf, wo_buf, q_buf, acc_ref, out_buf,
               x_sem, kv_sem, kv0_sem, wq_sem, wo_sem, out_sem):
        xt_hbm = (xta_hbm, xtb_hbm)
        k_hbm = (ka_hbm, kb_hbm)
        v_hbm = (va_hbm, vb_hbm)
        wq_hbm = (wqa_hbm, wqb_hbm)
        wot_hbm = (wota_hbm, wotb_hbm)

        def x_copy(blk):
            return pltpu.make_async_copy(xt_hbm[blk], xt_buf.at[blk], x_sem.at[blk])

        def k_copy(h, slot, blk):
            return pltpu.make_async_copy(k_hbm[blk].at[:, h], k_buf.at[slot, blk],
                                         kv_sem.at[slot, blk, 0])

        def v_copy(h, slot, blk):
            return pltpu.make_async_copy(v_hbm[blk].at[:, h], v_buf.at[slot, blk],
                                         kv_sem.at[slot, blk, 1])

        def kv0_copies(ci):
            b0, b1 = chunks[ci], chunks[ci + 1]
            out = []
            for blk in (0, 1):
                out.append(pltpu.make_async_copy(
                    k_hbm[blk].at[pl.ds(b0, b1 - b0), 0],
                    k_buf.at[0, blk, pl.ds(b0, b1 - b0)], kv0_sem.at[ci, blk, 0]))
                out.append(pltpu.make_async_copy(
                    v_hbm[blk].at[pl.ds(b0, b1 - b0), 0],
                    v_buf.at[0, blk, pl.ds(b0, b1 - b0)], kv0_sem.at[ci, blk, 1]))
            return out

        def wq_copy(h, slot, blk):
            return pltpu.make_async_copy(
                wq_hbm[blk].at[:, pl.ds(pl.multiple_of(h * W, W), W)],
                wq_buf.at[slot, blk], wq_sem.at[slot, blk])

        def wo_copy(h, slot, blk):
            return pltpu.make_async_copy(
                wot_hbm[blk].at[:, pl.ds(pl.multiple_of(h * W, W), W)],
                wo_buf.at[slot, blk], wo_sem.at[slot, blk])

        def out_copy(j):
            return pltpu.make_async_copy(out_buf.at[pl.ds(j * Sq, Sq)],
                                         out_hbm.at[pl.ds(j * Sq, Sq)], out_sem.at[j])

        def qproj(slot, blk, ci):
            q = jnp.dot(x_buf[blk, ci * MC:(ci + 1) * MC, :], wq_buf[slot, blk],
                        preferred_element_type=jnp.float32)
            q_buf[slot, blk, ci * MC:(ci + 1) * MC, :] = (q * c).astype(q_buf.dtype)

        def qk(slot, blk, j):
            qs = jnp.concatenate(
                [q_buf[slot, blk, j * Sq:(j + 1) * Sq, r * Dh:(r + 1) * Dh]
                 for r in range(rep)], axis=0)
            return lax.dot_general(qs, k_buf[slot, blk, j], _NT,
                                   preferred_element_type=jnp.float32)

        def softmax(s):
            m = jnp.max(s, axis=-1, keepdims=True)
            p = jnp.exp2(s - m)
            l = jnp.sum(p, axis=-1, keepdims=True)
            return p.astype(v_buf.dtype), l

        def pv(p, l, slot, blk, j):
            o = jnp.dot(p, v_buf[slot, blk, j], preferred_element_type=jnp.float32)
            o = (o / l).astype(wo_buf.dtype)
            return jnp.concatenate(
                [o[r * Sq:(r + 1) * Sq] for r in range(rep)], axis=1)

        def oproj(o, slot, blk, j, split):
            ds = D // split
            for t in range(split):
                acc_ref[blk * D + t * ds:blk * D + (t + 1) * ds, j * Sq:(j + 1) * Sq] += (
                    lax.dot_general(wo_buf[slot, blk, t * ds:(t + 1) * ds, :], o, _NT,
                                    preferred_element_type=jnp.float32))

        def emit_out(j):
            out_buf[j * Sq:(j + 1) * Sq, :] = (
                acc_ref[:, j * Sq:(j + 1) * Sq].T.astype(out_buf.dtype))
            out_copy(j).start()

        units = [(blk, j) for j in range(B) for blk in (0, 1)]
        n = len(units)

        def start_next(h, slot):
            for blk in (0, 1):
                k_copy(h + 1, 1 - slot, blk).start()
                v_copy(h + 1, 1 - slot, blk).start()
                wo_copy(h + 1, 1 - slot, blk).start()

            @pl.when(h + 2 < n_h)
            def _():
                for blk in (0, 1):
                    wq_copy(h + 2, slot, blk).start()

        def head(h, slot, first, last):
            if first:
                for cp in kv0_copies(0):
                    cp.wait()
            else:
                for blk in (0, 1):
                    k_copy(h, slot, blk).wait()
                    v_copy(h, slot, blk).wait()
            for blk in (0, 1):
                wo_copy(h, slot, blk).wait()
            if not last:
                for blk in (0, 1):
                    wq_copy(h + 1, 1 - slot, blk).wait()

            def qplan(pos):
                if not last:
                    for (p_, blk, ci) in _QPLAN:
                        if p_ == pos:
                            qproj(1 - slot, blk, ci)

            pend = []

            def flush(keep):
                while len(pend) > keep:
                    o_, uu = pend.pop(0)
                    oproj(o_, slot, *units[uu],
                          split=(2 if (last and uu >= n - _OSL) else 1))
                    if last and units[uu][0] == 1:
                        emit_out(units[uu][1])

            s = {0: qk(slot, *units[0])}
            for u in range(n):
                if u + 1 < n:
                    blk1, j1 = units[u + 1]
                    if first and blk1 == 0 and j1 in chunks[1:-1]:
                        for cp in kv0_copies(chunks.index(j1)):
                            cp.wait()
                    s[u + 1] = qk(slot, blk1, j1)
                p, l = softmax(s.pop(u))
                flush(_OD - 1)
                qplan(2 * u)
                if not last and u == _DMA_POS:
                    start_next(h, slot)
                pend.append((pv(p, l, slot, *units[u]), u))
                qplan(2 * u + 1)
            flush(0)
            qplan(2 * n)

        for blk in (0, 1):
            x_copy(blk).start()
            wq_copy(0, 0, blk).start()
        acc_ref[...] = jnp.zeros(acc_ref.shape, jnp.float32)
        x_copy(0).wait()
        for cp in kv0_copies(0):
            cp.start()
        for blk in (0, 1):
            wo_copy(0, 0, blk).start()
        for blk in (0, 1):
            wq_copy(1, 1, blk).start()
        for blk in (0, 1):
            if blk == 1:
                x_copy(blk).wait()
                for ci in range(1, n_ch):
                    for cp in kv0_copies(ci):
                        cp.start()
            wq_copy(0, 0, blk).wait()
            for ci in range(_NQ):
                for j in range(ci * B // _NQ, (ci + 1) * B // _NQ):
                    x_buf[blk, j * Sq:(j + 1) * Sq, :] = xt_buf[blk, j].T
                qproj(0, blk, ci)

        head(0, 0, True, False)

        def body(h, carry):
            head(h, lax.rem(h, 2), False, False)
            return carry

        lax.fori_loop(1, n_h - 1, body, 0)
        head(n_h - 1, (n_h - 1) % 2, False, True)
        for j in range(B):
            out_copy(j).wait()

    return kernel


@jax.jit
def pallas_concat_heads__gqa_block_cached__gqa_block_cached__near_ridge_kernel(
    A_x: jax.Array,
    A_k_cache: jax.Array,
    A_v_cache: jax.Array,
    A_wq: jax.Array,
    A_wo: jax.Array,
    B_x: jax.Array,
    B_k_cache: jax.Array,
    B_v_cache: jax.Array,
    B_wq: jax.Array,
    B_wo: jax.Array,
):
    B, Sq, D = A_x.shape
    _, Hkv, Sk, Dh = A_k_cache.shape
    Hq = A_wq.shape[1] // Dh
    rep = Hq // Hkv
    W = rep * Dh
    dt = A_x.dtype

    xta = jnp.transpose(A_x, (0, 2, 1))
    xtb = jnp.transpose(B_x, (0, 2, 1))
    wota = A_wo.T
    wotb = B_wo.T

    any_spec = pl.BlockSpec(memory_space=pl.ANY)
    out = pl.pallas_call(
        _make_kernel(B, Sq, D, Sk, Dh, rep, Hkv),
        in_specs=[any_spec] * 10,
        out_specs=any_spec,
        out_shape=jax.ShapeDtypeStruct((B * Sq, 2 * D), dt),
        scratch_shapes=[
            pltpu.VMEM((2, B, D, Sq), dt),
            pltpu.VMEM((2, B * Sq, D), dt),
            pltpu.VMEM((2, 2, B, Sk, Dh), dt),
            pltpu.VMEM((2, 2, B, Sk, Dh), dt),
            pltpu.VMEM((2, 2, D, W), dt),
            pltpu.VMEM((2, 2, D, W), dt),
            pltpu.VMEM((2, 2, B * Sq, W), dt),
            pltpu.VMEM((2 * D, B * Sq), jnp.float32),
            pltpu.VMEM((B * Sq, 2 * D), dt),
            pltpu.SemaphoreType.DMA((2,)),
            pltpu.SemaphoreType.DMA((2, 2, 2)),
            pltpu.SemaphoreType.DMA((len(_CHUNKS) - 1, 2, 2)),
            pltpu.SemaphoreType.DMA((2, 2)),
            pltpu.SemaphoreType.DMA((2, 2)),
            pltpu.SemaphoreType.DMA((B,)),
        ],
        compiler_params=pltpu.CompilerParams(
            vmem_limit_bytes=100 * 1024 * 1024,
            disable_bounds_checks=True),
    )(xta, A_k_cache, A_v_cache, A_wq, wota,
      xtb, B_k_cache, B_v_cache, B_wq, wotb)
    return out.reshape(B, Sq, 2 * D)
```

```python
import functools
import math

import jax
import jax.numpy as jnp
from jax import lax
import jax.experimental.pallas as pl
import jax.experimental.pallas.tpu as pltpu

_NT = (((1,), (1,)), ((), ()))

_NQ = 4
_QPLAN = ((26, 0, 0), (27, 0, 1), (28, 0, 2), (29, 0, 3),
          (30, 1, 0), (31, 1, 1), (32, 1, 2), (32, 1, 3))
_DMA_POS = 4
_CHUNKS = (0, 2, 5, 8)
_OD = 2
_OSL = 2


def _make_kernel(B, Sq, D, Sk, Dh, rep, n_h):
    c = (Dh ** -0.5) * math.log2(math.e)
    M = B * Sq
    W = rep * Dh
    MC = M // _NQ
    chunks = _CHUNKS
    n_ch = len(chunks) - 1

    def kernel(xta_hbm, ka_hbm, va_hbm, wqa_hbm, wota_hbm,
               xtb_hbm, kb_hbm, vb_hbm, wqb_hbm, wotb_hbm,
               out_hbm,
               xt_buf, x_buf, k_buf, v_buf, wq_buf, wo_buf, q_buf, acc_ref, out_buf,
               x_sem, kv_sem, kv0_sem, wq_sem, wo_sem, out_sem):
        xt_hbm = (xta_hbm, xtb_hbm)
        k_hbm = (ka_hbm, kb_hbm)
        v_hbm = (va_hbm, vb_hbm)
        wq_hbm = (wqa_hbm, wqb_hbm)
        wot_hbm = (wota_hbm, wotb_hbm)

        def x_copy(blk):
            return pltpu.make_async_copy(xt_hbm[blk], xt_buf.at[blk], x_sem.at[blk])

        def k_copy(h, slot, blk):
            return pltpu.make_async_copy(k_hbm[blk].at[:, h], k_buf.at[slot, blk],
                                         kv_sem.at[slot, blk, 0])

        def v_copy(h, slot, blk):
            return pltpu.make_async_copy(v_hbm[blk].at[:, h], v_buf.at[slot, blk],
                                         kv_sem.at[slot, blk, 1])

        def kv0_copies(ci):
            b0, b1 = chunks[ci], chunks[ci + 1]
            out = []
            for blk in (0, 1):
                out.append(pltpu.make_async_copy(
                    k_hbm[blk].at[pl.ds(b0, b1 - b0), 0],
                    k_buf.at[0, blk, pl.ds(b0, b1 - b0)], kv0_sem.at[ci, blk, 0]))
                out.append(pltpu.make_async_copy(
                    v_hbm[blk].at[pl.ds(b0, b1 - b0), 0],
                    v_buf.at[0, blk, pl.ds(b0, b1 - b0)], kv0_sem.at[ci, blk, 1]))
            return out

        def wq_copy(h, slot, blk):
            return pltpu.make_async_copy(
                wq_hbm[blk].at[:, pl.ds(pl.multiple_of(h * W, W), W)],
                wq_buf.at[slot, blk], wq_sem.at[slot, blk])

        def wo_copy(h, slot, blk):
            return pltpu.make_async_copy(
                wot_hbm[blk].at[:, pl.ds(pl.multiple_of(h * W, W), W)],
                wo_buf.at[slot, blk], wo_sem.at[slot, blk])

        def out_copy(j):
            return pltpu.make_async_copy(out_buf.at[pl.ds(j * Sq, Sq)],
                                         out_hbm.at[pl.ds(j * Sq, Sq)], out_sem.at[j])

        def qproj(slot, blk, ci):
            q = jnp.dot(x_buf[blk, ci * MC:(ci + 1) * MC, :], wq_buf[slot, blk],
                        preferred_element_type=jnp.float32)
            q_buf[slot, blk, ci * MC:(ci + 1) * MC, :] = (q * c).astype(q_buf.dtype)

        def qk(slot, blk, j):
            qs = jnp.concatenate(
                [q_buf[slot, blk, j * Sq:(j + 1) * Sq, r * Dh:(r + 1) * Dh]
                 for r in range(rep)], axis=0)
            return lax.dot_general(qs, k_buf[slot, blk, j], _NT,
                                   preferred_element_type=jnp.float32)

        def softmax(s):
            m = jnp.max(s, axis=-1, keepdims=True)
            p = jnp.exp2(s - m)
            l = jnp.sum(p, axis=-1, keepdims=True)
            return p.astype(v_buf.dtype), l

        def pv(p, l, slot, blk, j):
            o = jnp.dot(p, v_buf[slot, blk, j], preferred_element_type=jnp.float32)
            o = (o / l).astype(wo_buf.dtype)
            return jnp.concatenate(
                [o[r * Sq:(r + 1) * Sq] for r in range(rep)], axis=1)

        def oproj(o, slot, blk, j, split):
            ds = D // split
            for t in range(split):
                acc_ref[blk * D + t * ds:blk * D + (t + 1) * ds, j * Sq:(j + 1) * Sq] += (
                    lax.dot_general(wo_buf[slot, blk, t * ds:(t + 1) * ds, :], o, _NT,
                                    preferred_element_type=jnp.float32))

        def emit_out(j):
            out_buf[j * Sq:(j + 1) * Sq, :] = (
                acc_ref[:, j * Sq:(j + 1) * Sq].T.astype(out_buf.dtype))
            out_copy(j).start()

        units = [(blk, j) for j in range(B) for blk in (0, 1)]
        n = len(units)

        def start_next(h, slot):
            for blk in (0, 1):
                k_copy(h + 1, 1 - slot, blk).start()
                v_copy(h + 1, 1 - slot, blk).start()
                wo_copy(h + 1, 1 - slot, blk).start()

            @pl.when(h + 2 < n_h)
            def _():
                for blk in (0, 1):
                    wq_copy(h + 2, slot, blk).start()

        def head(h, slot, first, last):
            if first:
                for cp in kv0_copies(0):
                    cp.wait()
            else:
                for blk in (0, 1):
                    k_copy(h, slot, blk).wait()
                    v_copy(h, slot, blk).wait()
            for blk in (0, 1):
                wo_copy(h, slot, blk).wait()
            if not last and not first:
                for blk in (0, 1):
                    wq_copy(h + 1, 1 - slot, blk).wait()

            def qplan(pos):
                if not last:
                    for (p_, blk, ci) in _QPLAN:
                        if p_ == pos:
                            qproj(1 - slot, blk, ci)

            pend = []

            def flush(keep):
                while len(pend) > keep:
                    o_, uu = pend.pop(0)
                    oproj(o_, slot, *units[uu],
                          split=(2 if (last and uu >= n - _OSL) else 1))
                    if last and units[uu][0] == 1:
                        emit_out(units[uu][1])

            s = {0: qk(slot, *units[0])}
            for u in range(n):
                if u + 1 < n:
                    blk1, j1 = units[u + 1]
                    if first and blk1 == 0 and j1 in chunks[1:-1]:
                        for cp in kv0_copies(chunks.index(j1)):
                            cp.wait()
                        if j1 == chunks[-2]:
                            for blk in (0, 1):
                                wq_copy(h + 1, 1 - slot, blk).wait()
                    s[u + 1] = qk(slot, blk1, j1)
                p, l = softmax(s.pop(u))
                flush(_OD - 1)
                qplan(2 * u)
                if not last and u == _DMA_POS:
                    start_next(h, slot)
                pend.append((pv(p, l, slot, *units[u]), u))
                qplan(2 * u + 1)
            flush(0)
            qplan(2 * n)

        for blk in (0, 1):
            x_copy(blk).start()
            wq_copy(0, 0, blk).start()
        acc_ref[...] = jnp.zeros(acc_ref.shape, jnp.float32)
        x_copy(0).wait()
        for cp in kv0_copies(0):
            cp.start()
        for blk in (0, 1):
            wo_copy(0, 0, blk).start()
        for blk in (0, 1):
            if blk == 1:
                x_copy(blk).wait()
                for ci in range(1, n_ch):
                    for cp in kv0_copies(ci):
                        cp.start()
                for b2 in (0, 1):
                    wq_copy(1, 1, b2).start()
            wq_copy(0, 0, blk).wait()
            for ci in range(_NQ):
                for j in range(ci * B // _NQ, (ci + 1) * B // _NQ):
                    x_buf[blk, j * Sq:(j + 1) * Sq, :] = xt_buf[blk, j].T
                qproj(0, blk, ci)

        head(0, 0, True, False)

        def body(h, carry):
            head(h, lax.rem(h, 2), False, False)
            return carry

        lax.fori_loop(1, n_h - 1, body, 0)
        head(n_h - 1, (n_h - 1) % 2, False, True)
        for j in range(B):
            out_copy(j).wait()

    return kernel


@jax.jit
def pallas_concat_heads__gqa_block_cached__gqa_block_cached__near_ridge_kernel(
    A_x: jax.Array,
    A_k_cache: jax.Array,
    A_v_cache: jax.Array,
    A_wq: jax.Array,
    A_wo: jax.Array,
    B_x: jax.Array,
    B_k_cache: jax.Array,
    B_v_cache: jax.Array,
    B_wq: jax.Array,
    B_wo: jax.Array,
):
    B, Sq, D = A_x.shape
    _, Hkv, Sk, Dh = A_k_cache.shape
    Hq = A_wq.shape[1] // Dh
    rep = Hq // Hkv
    W = rep * Dh
    dt = A_x.dtype

    xta = jnp.transpose(A_x, (0, 2, 1))
    xtb = jnp.transpose(B_x, (0, 2, 1))
    wota = A_wo.T
    wotb = B_wo.T

    any_spec = pl.BlockSpec(memory_space=pl.ANY)
    out = pl.pallas_call(
        _make_kernel(B, Sq, D, Sk, Dh, rep, Hkv),
        in_specs=[any_spec] * 10,
        out_specs=any_spec,
        out_shape=jax.ShapeDtypeStruct((B * Sq, 2 * D), dt),
        scratch_shapes=[
            pltpu.VMEM((2, B, D, Sq), dt),
            pltpu.VMEM((2, B * Sq, D), dt),
            pltpu.VMEM((2, 2, B, Sk, Dh), dt),
            pltpu.VMEM((2, 2, B, Sk, Dh), dt),
            pltpu.VMEM((2, 2, D, W), dt),
            pltpu.VMEM((2, 2, D, W), dt),
            pltpu.VMEM((2, 2, B * Sq, W), dt),
            pltpu.VMEM((2 * D, B * Sq), jnp.float32),
            pltpu.VMEM((B * Sq, 2 * D), dt),
            pltpu.SemaphoreType.DMA((2,)),
            pltpu.SemaphoreType.DMA((2, 2, 2)),
            pltpu.SemaphoreType.DMA((len(_CHUNKS) - 1, 2, 2)),
            pltpu.SemaphoreType.DMA((2, 2)),
            pltpu.SemaphoreType.DMA((2, 2)),
            pltpu.SemaphoreType.DMA((B,)),
        ],
        compiler_params=pltpu.CompilerParams(
            vmem_limit_bytes=100 * 1024 * 1024,
            disable_bounds_checks=True),
    )(xta, A_k_cache, A_v_cache, A_wq, wota,
      xtb, B_k_cache, B_v_cache, B_wq, wotb)
    return out.reshape(B, Sq, 2 * D)
```
